```python
import jax
import jax.numpy as jnp

def _softmax(x, axis=-1):
    return jax.nn.softmax(x, axis=axis)

def _gelu(x):
    return jax.nn.gelu(x, approximate=True)

def _silu(x):
    return jax.nn.silu(x)

def _sigmoid(x):
    return jax.nn.sigmoid(x)

def _layernorm(x, axis=-1, eps=1e-05):
    m = jnp.mean(x, axis=axis, keepdims=True)
    v = jnp.var(x, axis=axis, keepdims=True)
    return (x - m) / jnp.sqrt(v + eps)

def _scatter_add(tgt, idx, src, axis=0):
    return tgt.at[idx].add(src)

def _segment_sum(src, seg, n):
    return jax.ops.segment_sum(src, seg, n)

class _Rng:

    def __init__(self, key):
        self._k = key

    def _next(self):
        self._k, sub = jax.random.split(self._k)
        return sub

    def normal(self, shape):
        return jax.random.normal(self._next(), shape, dtype=jnp.bfloat16)

    def randint(self, lo, hi, shape):
        return jax.random.randint(self._next(), shape, lo, hi, dtype=jnp.int32)

    def uniform(self, shape, lo=0.0, hi=1.0):
        return jax.random.uniform(self._next(), shape, jnp.bfloat16, lo, hi)

    def permutation(self, n):
        return jax.random.permutation(self._next(), n)
kernel_name = 'adaLN_cond__sliding_block_cached__dense_activation_mish__decode'

def setup_inputs():
    _rng = _Rng(jax.random.key(int.from_bytes(__import__("os").urandom(4), "little")))
    _w = lambda a: (lambda t: t.astype(jnp.bfloat16) if jnp.issubdtype(t.dtype, jnp.floating) else t)(jnp.asarray(a))

    def _A_setup():
        B, Sq, D = (1, 1, 640)
        Hq, Hkv, Sk, Dh = (32, 32, 32768, 192)
        assert Hq % Hkv == 0, (Hq, Hkv)
        return {'x': _w((lambda *s: _rng.normal(s) * 0.05)(B, Sq, D)), 'k_cache': _w((lambda *s: _rng.normal(s) * 0.05)(B, Hkv, Sk, Dh)), 'v_cache': _w((lambda *s: _rng.normal(s) * 0.05)(B, Hkv, Sk, Dh)), 'wq': _w((lambda *s: _rng.normal(s) * 0.05)(D, Hq * Dh) * D ** (-0.5)), 'wo': _w((lambda *s: _rng.normal(s) * 0.05)(Hq * Dh, D) * (Hq * Dh) ** (-0.5))}
    _A_in = _A_setup()

    def _B_setup():
        B, S, D, F = (1, 1, 640, 1536)
        return {'x': _w((lambda *s: _rng.normal(s) * 0.05)(B, S, D)), 'w1': _w((lambda *s: _rng.normal(s) * 0.05)(D, F) * D ** (-0.5)), 'b1': _w((lambda *s: _rng.normal(s) * 0.05)(F)), 'w2': _w((lambda *s: _rng.normal(s) * 0.05)(F, D) * F ** (-0.5))}
    _B_in = _B_setup()
    return {'A_x': _A_in['x'], 'A_k_cache': _A_in['k_cache'], 'A_v_cache': _A_in['v_cache'], 'A_wq': _A_in['wq'], 'A_wo': _A_in['wo'], 'B_x': _B_in['x'], 'B_w1': _B_in['w1'], 'B_b1': _B_in['b1'], 'B_w2': _B_in['w2'], 'c': _w((lambda *s: _rng.normal(s) * 0.05)(1, 640)), 'w_mod': _w((lambda *s: _rng.normal(s) * 0.05)(640, 6 * 640) * 640 ** (-0.5))}

def reference(A_x, A_k_cache, A_v_cache, A_wq, A_wo, B_x, B_w1, B_b1, B_w2, c, w_mod):

    def _A_ref(x, k_cache, v_cache, wq, wo):
        B, Sq, D = x.shape
        Hq, Dh = (32, 192)
        Hkv, Sk = (k_cache.shape[1], k_cache.shape[2])
        W = min(4096, max(256, Sk // 4))
        rep = Hq // Hkv
        q = (lambda x, *d: x.transpose(*d))((x @ wq).reshape(B, Sq, Hq, Dh), 0, 2, 1, 3)
        k = jnp.repeat(k_cache[:, :, Sk - W:, :], rep, axis=1)
        v = jnp.repeat(v_cache[:, :, Sk - W:, :], rep, axis=1)
        scores = jnp.einsum('bhqd,bhkd->bhqk', q, k) * Dh ** (-0.5)
        p = _softmax(scores, axis=-1)
        o = jnp.einsum('bhqk,bhkd->bhqd', p, v)
        return (lambda x, *d: x.transpose(*d))(o, 0, 2, 1, 3).reshape(B, Sq, Hq * Dh) @ wo

    def _B_ref(x, w1, b1, w2):
        h = jnp.einsum('bsd,df->bsf', x, w1) + b1
        sp = jnp.log1p(jnp.exp(-jnp.abs(h))) + jnp.where(h > 0, h, jnp.zeros_like(h))
        act = h * jnp.tanh(sp)
        return jnp.einsum('bsf,fd->bsd', act, w2)
    x = A_x
    mod = (_silu(c) @ w_mod).reshape(c.shape[0], 6, 1, -1)
    sa, ca, ga, sb, cb, gb = (mod[:, 0].copy(), mod[:, 1].copy(), mod[:, 2].copy(), mod[:, 3].copy(), mod[:, 4].copy(), mod[:, 5].copy())
    h = _layernorm(x, axis=-1) * (1 + ca) + sa
    x = x + ga * _A_ref(h, A_k_cache, A_v_cache, A_wq, A_wo)
    h = _layernorm(x, axis=-1) * (1 + cb) + sb
    x = x + gb * _B_ref(h, B_w1, B_b1, B_w2)
    return x
```

```python
import functools

import jax
import jax.numpy as jnp
from jax import lax
import jax.experimental.pallas as pl
import jax.experimental.pallas.tpu as pltpu

F32 = jnp.float32
BF16 = jnp.bfloat16

D = 640
H = 32
DH = 192
FF = 1536
EPS = 1e-5
RC = 16
NT = DH // RC
PAIR = 2 * DH
WQ_RB = 32
WQ_N = D // 2 // WQ_RB
LO, HI = 1, 0
SLAB = 512


def _layernorm(x):
    m = jnp.mean(x, axis=-1, keepdims=True)
    xc = x - m
    v = jnp.mean(xc * xc, axis=-1, keepdims=True)
    return xc / jnp.sqrt(v + EPS)


def _kernel(x_hbm, c_hbm, b1_hbm, k_hbm, v_hbm, wq_hbm, wo_hbm, w1_hbm, w2_hbm,
            wm_hbm, o_ref,
            x_v, c_v, b1_v, kbuf, vbuf, wq_v, wo_v, w1_v, w2_v, wm_v,
            h_s, sc_s, qb_s, s_s, p_s, acc_s, mod_s,
            ksem, vsem, wsem, *, win, start):

    def k_copy(h, r):
        rows = pl.ds(pl.multiple_of(r * RC, RC), RC)
        return pltpu.make_async_copy(
            k_hbm.at[0, h, rows, pl.ds(start, win)], kbuf.at[rows, :], ksem.at[r])

    def v_copy(h, r):
        rows = pl.ds(pl.multiple_of(r * RC, RC), RC)
        return pltpu.make_async_copy(
            v_hbm.at[0, h, rows, pl.ds(start, win)], vbuf.at[rows, :], vsem.at[r])

    def w2_copy(r):
        rows = pl.ds(pl.multiple_of(r * 128, 128), 128)
        return pltpu.make_async_copy(
            w2_hbm.at[rows, :], w2_v.at[rows, :], ksem.at[r])

    def whole(ref, sem):
        return pltpu.make_async_copy(ref, ref, sem)

    cp_c = pltpu.make_async_copy(c_hbm, c_v, wsem.at[1])
    cp_x = pltpu.make_async_copy(x_hbm, x_v, wsem.at[0])
    cp_b1 = pltpu.make_async_copy(b1_hbm, b1_v, wsem.at[2])
    cp_wma = pltpu.make_async_copy(
        wm_hbm.at[:, pl.ds(0, 2 * D)], wm_v.at[:, pl.ds(0, 2 * D)], wsem.at[3])
    cp_wmg = pltpu.make_async_copy(
        wm_hbm.at[:, pl.ds(2 * D, D)], wm_v.at[:, pl.ds(2 * D, D)], wsem.at[4])
    cp_wq0 = pltpu.make_async_copy(
        wq_hbm.at[:, pl.ds(0, PAIR)], wq_v, wsem.at[6])
    cp_wo0 = pltpu.make_async_copy(
        wo_hbm.at[pl.ds(0, DH), :], wo_v.at[0], wsem.at[7])
    cp_wma.start(priority=HI)
    cp_c.start(priority=HI)
    cp_x.start(priority=HI)
    cp_wq0.start(priority=HI)
    for r in range(NT):
        k_copy(0, r).start(priority=LO)
    cp_wo0.start(priority=HI)
    cp_wmg.start(priority=HI)
    cp_b1.start(priority=HI)

    acc_s[...] = jnp.zeros_like(acc_s)

    cp_c.wait()
    cp_x.wait()
    c = c_v[...].astype(F32)
    sc = c * (1.0 / (1.0 + jnp.exp(-c)))
    sc_s[...] = jnp.broadcast_to(sc, sc_s.shape).astype(BF16)
    xn = _layernorm(x_v[0].astype(F32))
    cp_wma.wait()
    mod_a = jnp.dot(sc_s[...], wm_v[:, 0:2 * D], preferred_element_type=F32)
    h1 = xn * (1.0 + mod_a[:, D:2 * D]) + mod_a[:, 0:D]
    h_s[...] = h1.astype(BF16)

    def q_prep():
        whole(wq_v, wsem.at[6]).wait()
        q = jnp.dot(h_s[...], wq_v[...], preferred_element_type=F32)
        q = q[0:1, :] * (DH ** -0.5)
        for b in range(PAIR // 128):
            qb_s[b * 128:(b + 1) * 128, :] = jnp.broadcast_to(
                q[:, b * 128:(b + 1) * 128], (128, 128)).T

    q_prep()

    def head(h, carry):
        par = lax.rem(h, 2)
        s_s[...] = jnp.zeros_like(s_s)

        def k_tick(r, c_):
            k_copy(h, r).wait()
            v_copy(h, r).start(priority=LO)

            @pl.when(r < WQ_N)
            def _():
                rows = pl.ds(pl.multiple_of(par * (D // 2) + r * WQ_RB, WQ_RB), WQ_RB)

                @pl.when(h < H - 2)
                def _():
                    col = pl.multiple_of((lax.div(h, 2) + 1) * PAIR, 128)
                    pltpu.make_async_copy(
                        wq_hbm.at[rows, pl.ds(col, PAIR)], wq_v.at[rows, :],
                        wsem.at[6]).start(priority=HI)

                @pl.when(h >= H - 2)
                def _():
                    pltpu.make_async_copy(
                        w1_hbm.at[rows, :], w1_v.at[rows, :],
                        wsem.at[9]).start(priority=HI)

            @pl.when(jnp.logical_and(r >= WQ_N, h < H - 2))
            def _():
                n = 2 * h + (r - WQ_N)
                rows = pl.ds(pl.multiple_of(lax.rem(n, 20) * 32, 32), 32)
                cols = pl.ds(pl.multiple_of((3 + lax.div(n, 20)) * D, 128), D)
                pltpu.make_async_copy(
                    wm_hbm.at[rows, cols], wm_v.at[rows, cols],
                    wsem.at[5]).start(priority=HI)

            rows = pl.ds(pl.multiple_of(r * RC, RC), RC)
            qb = qb_s[pl.ds(pl.multiple_of(par * DH + r * RC, RC), RC), :]
            qb = jnp.concatenate([qb] * (SLAB // 128), axis=1)
            for j in range(win // SLAB):
                cols = slice(j * SLAB, (j + 1) * SLAB)
                pr = kbuf[rows, cols].astype(F32) * qb
                s_s[:, cols] += pr[0:8] + pr[8:16]
            return c_

        lax.fori_loop(0, NT, k_tick, 0)

        s = jnp.sum(s_s[...], axis=0, keepdims=True)
        m = jnp.max(s, axis=1, keepdims=True)
        p = jnp.exp(s - m)
        inv_l = 1.0 / jnp.sum(p, axis=1, keepdims=True)
        p_s[...] = jnp.broadcast_to(p, p_s.shape)
        whole(wo_v.at[par], wsem.at[7 + par]).wait()

        def v_tick(r, c_):
            v_copy(h, r).wait()
            rows = pl.ds(pl.multiple_of(r * RC, RC), RC)

            @pl.when(h < H - 1)
            def _():
                k_copy(h + 1, r).start(priority=LO)
                pltpu.make_async_copy(
                    wo_hbm.at[pl.ds(pl.multiple_of((h + 1) * DH + r * RC, RC), RC), :],
                    wo_v.at[1 - par, rows, :],
                    wsem.at[8 - par]).start(priority=HI)

            @pl.when(h == H - 1)
            def _():
                w2_copy(r).start(priority=LO)

            a0 = jnp.zeros((8, SLAB), F32)
            a1 = jnp.zeros((8, SLAB), F32)
            for j in range(win // SLAB):
                cols = slice(j * SLAB, (j + 1) * SLAB)
                vt = vbuf[rows, cols].astype(F32)
                pj = p_s[:, cols]
                a0 = a0 + vt[0:8] * pj
                a1 = a1 + vt[8:16] * pj
            o0 = jnp.sum(a0, axis=1, keepdims=True) * inv_l
            o1 = jnp.sum(a1, axis=1, keepdims=True) * inv_l
            wo = wo_v[par, rows, :].astype(F32)
            acc_s[...] += wo[0:8] * o0 + wo[8:16] * o1
            return c_

        lax.fori_loop(0, NT, v_tick, 0)

        @pl.when(jnp.logical_and(par == 1, h < H - 1))
        def _():
            q_prep()

        @pl.when(h == H - 2)
        def _():
            cp_wmg.wait()
            whole(wm_v.at[:, pl.ds(3 * D, 3 * D)], wsem.at[5]).wait()
            mod_s[...] = jnp.dot(sc_s[...], wm_v[:, 2 * D:6 * D],
                                 preferred_element_type=F32)

        return carry

    lax.fori_loop(0, H, head, 0)

    attn = jnp.sum(acc_s[...], axis=0, keepdims=True)
    x1 = x_v[0].astype(F32) + mod_s[0:1, 0:D] * attn
    h2 = _layernorm(x1) * (1.0 + mod_s[0:1, 2 * D:3 * D]) + mod_s[0:1, D:2 * D]
    h2 = jnp.broadcast_to(h2, (8, D)).astype(BF16)
    cp_b1.wait()
    whole(w1_v, wsem.at[9]).wait()
    u = jnp.dot(h2, w1_v[...], preferred_element_type=F32)
    u = u + b1_v[...].astype(F32).reshape(1, FF)
    sp = jnp.log1p(jnp.exp(-jnp.abs(u))) + jnp.where(u > 0, u, 0.0)
    act = (u * jnp.tanh(sp)).astype(BF16)
    y = jnp.zeros((8, D), F32)
    for r in range(NT):
        w2_copy(r).wait()
        y = y + jnp.dot(act[:, r * 128:(r + 1) * 128],
                        w2_v[r * 128:(r + 1) * 128, :],
                        preferred_element_type=F32)
    out = x1 + mod_s[0:1, 3 * D:4 * D] * y[0:1]
    o_ref[0] = out.astype(o_ref.dtype)


@jax.jit
def pallas_adaLN_cond__sliding_block_cached__dense_activation_mish__decode_kernel(
    A_x: jax.Array,
    A_k_cache: jax.Array,
    A_v_cache: jax.Array,
    A_wq: jax.Array,
    A_wo: jax.Array,
    B_x: jax.Array,
    B_w1: jax.Array,
    B_b1: jax.Array,
    B_w2: jax.Array,
    c: jax.Array,
    w_mod: jax.Array,
):
    del B_x
    sk = A_k_cache.shape[2]
    win = min(4096, max(256, sk // 4))
    assert A_x.shape == (1, 1, D) and A_k_cache.shape == (1, H, sk, DH)
    assert FF // 128 == NT and win % SLAB == 0 and (sk - win) % 128 == 0
    kt = jnp.swapaxes(A_k_cache, 2, 3)
    vt = jnp.swapaxes(A_v_cache, 2, 3)

    any_spec = pl.BlockSpec(memory_space=pl.ANY)
    return pl.pallas_call(
        functools.partial(_kernel, win=win, start=sk - win),
        out_shape=jax.ShapeDtypeStruct((1, 1, D), A_x.dtype),
        in_specs=[any_spec] * 10,
        out_specs=pl.BlockSpec(memory_space=pltpu.VMEM),
        scratch_shapes=[
            pltpu.VMEM((1, 1, D), BF16),
            pltpu.VMEM((1, D), BF16),
            pltpu.VMEM((FF,), BF16),
            pltpu.VMEM((DH, win), BF16),
            pltpu.VMEM((DH, win), BF16),
            pltpu.VMEM((D, PAIR), BF16),
            pltpu.VMEM((2, DH, D), BF16),
            pltpu.VMEM((D, FF), BF16),
            pltpu.VMEM((FF, D), BF16),
            pltpu.VMEM((D, 6 * D), BF16),
            pltpu.VMEM((8, D), BF16),
            pltpu.VMEM((8, D), BF16),
            pltpu.VMEM((PAIR, 128), F32),
            pltpu.VMEM((8, win), F32),
            pltpu.VMEM((8, win), F32),
            pltpu.VMEM((8, D), F32),
            pltpu.VMEM((8, 4 * D), F32),
            pltpu.SemaphoreType.DMA((NT,)),
            pltpu.SemaphoreType.DMA((NT,)),
            pltpu.SemaphoreType.DMA((10,)),
        ],
        compiler_params=pltpu.CompilerParams(vmem_limit_bytes=64 * 1024 * 1024),
        name="adaln_decode",
    )(A_x, c, B_b1, kt, vt, A_wq, A_wo, B_w1, B_w2, w_mod)
```

```python
import functools

import jax
import jax.numpy as jnp
from jax import lax
import jax.experimental.pallas as pl
import jax.experimental.pallas.tpu as pltpu

F32 = jnp.float32
BF16 = jnp.bfloat16

D = 640
H = 32
DH = 192
FF = 1536
EPS = 1e-5
PAIR = 2 * DH
LO, HI = 1, 0
TN = 128
WQR = 32
NRB = D // WQR
NWQ = 3 * NRB // 2
NWO = DH // 16

CFG = dict(NWM=6, guard=4, tailg=(4, 4, 2), proticks=True, vputail=2, NL0=24, early=0)


def _layernorm(x):
    m = jnp.mean(x, axis=-1, keepdims=True)
    xc = x - m
    v = jnp.mean(xc * xc, axis=-1, keepdims=True)
    return xc / jnp.sqrt(v + EPS)


def _tree_sum(xs):
    xs = list(xs)
    while len(xs) > 1:
        xs = [xs[i] + xs[i + 1] if i + 1 < len(xs) else xs[i] for i in range(0, len(xs), 2)]
    return xs[0]


def _kernel(x_hbm, c_hbm, b1_hbm, k_hbm, v_hbm, wq_hbm, wo_hbm, w1_hbm, w2_hbm,
            wm_hbm, o_ref,
            x_v, c_v, b1_v, kbuf, vbuf, wq_v, wo_v, w1_v, w2_v, wm_v,
            h_s, sc_s, qb_s, s_s, acc_s, mod_s, ab_s,
            sem, psem, wsem, *, win, start, cfg):
    NWM = cfg['NWM']
    NP = win // TN
    T = 2 * NP
    WM_TOT = (D // 16) * 4
    WM_HEADS = -(-WM_TOT // NWM)
    W2_EARLY = min((H - WM_HEADS) * NWM, cfg.get('early', 10 ** 9))
    W2_G = FF // 16
    rem = W2_G - W2_EARLY
    tail = [rem // NP + (1 if i < rem % NP else 0) for i in range(NP)]
    if cfg.get('tailsplit'):
        tail = list(cfg['tailsplit']) + [0] * (NP - len(cfg['tailsplit']))
        assert sum(tail) == rem, (sum(tail), rem)
    tail_off = [W2_EARLY + sum(tail[:i]) for i in range(NP)]

    def kv_copy(src, buf, h, j):
        return pltpu.make_async_copy(
            src.at[0, h, :, pl.ds(start + j * TN, TN)], buf.at[j], sem.at[j])

    k_copy = functools.partial(kv_copy, k_hbm, kbuf)
    v_copy = functools.partial(kv_copy, v_hbm, vbuf)

    def w2_tail(i):
        rows = pl.ds(tail_off[i] * 16, tail[i] * 16)
        return pltpu.make_async_copy(w2_hbm.at[rows, :], w2_v.at[rows, :], sem.at[i])

    def whole(ref, s):
        return pltpu.make_async_copy(ref, ref, s)

    items = []
    for nm, k in (('wq', NWQ), ('wo', NWO), ('wm', NWM)):
        items += [((i + 0.5) / k, nm) for i in range(k)]
    kinds = [nm for _, nm in sorted(items)]
    last_ok = T - cfg['guard']
    slots, cnt = {}, {'wq': 0, 'wo': 0, 'wm': 0}
    for i, kd in enumerate(kinds):
        slots.setdefault((i * last_ok) // len(kinds), []).append((kd, cnt[kd]))
        cnt[kd] += 1

    cp_c = pltpu.make_async_copy(c_hbm, c_v, wsem.at[1])
    cp_x = pltpu.make_async_copy(x_hbm, x_v, wsem.at[0])
    cp_b1 = pltpu.make_async_copy(b1_hbm, b1_v, wsem.at[2])

    def small_prep():
        acc_s[...] = jnp.zeros_like(acc_s)
        cp_c.wait()
        cp_x.wait()
        c = c_v[...].astype(F32)
        sc = c * (1.0 / (1.0 + jnp.exp(-c)))
        sc_s[...] = jnp.broadcast_to(sc, sc_s.shape).astype(BF16)
        return _layernorm(x_v[0].astype(F32))

    if not cfg['proticks']:
        cp_wma = pltpu.make_async_copy(
            wm_hbm.at[:, pl.ds(0, 2 * D)], wm_v.at[:, pl.ds(0, 2 * D)], wsem.at[3])
        cp_wq0 = pltpu.make_async_copy(
            wq_hbm.at[:, pl.ds(0, PAIR)], wq_v, wsem.at[6])
        cp_c.start(priority=HI)
        cp_x.start(priority=HI)
        cp_wma.start(priority=HI)
        cp_wq0.start(priority=HI)
        cp_b1.start(priority=HI)
        for j in range(NP):
            k_copy(0, j).start(priority=LO)
        xn = small_prep()
        cp_wma.wait()
    else:
        NA = D // 16
        NL0 = cfg['NL0']

        def wma_copy(i):
            rows = pl.ds(i * 16, 16)
            cols = pl.ds(0, 2 * D)
            return pltpu.make_async_copy(wm_hbm.at[rows, cols], wm_v.at[rows, cols],
                                         psem.at[i])

        def wq0_copy(m):
            rows = pl.ds((m % NRB) * WQR, WQR)
            cols = pl.ds((m // NRB) * 128, 128)
            return pltpu.make_async_copy(wq_hbm.at[rows, cols], wq_v.at[rows, cols],
                                         wsem.at[6])
        lows = [functools.partial(wma_copy, i) for i in range(NA)]
        lows += [functools.partial(k_copy, 0, j) for j in range(NP)]
        cp_c.start(priority=HI)
        cp_x.start(priority=HI)
        for f in lows[:NL0]:
            f().start(priority=LO)
        cp_b1.start(priority=HI)
        nxt = NL0
        m = 0
        for i in range(NA):
            wma_copy(i).wait()
            upto = NL0 + ((i + 1) * (len(lows) - NL0)) // NA
            while nxt < upto:
                lows[nxt]().start(priority=LO)
                nxt += 1
            while m < ((i + 1) * 3 * NRB) // (NA - 4) and m < 3 * NRB:
                wq0_copy(m).start(priority=HI)
                m += 1
            if i == cfg.get('prepat', 8):
                xn = small_prep()
        assert nxt == len(lows) and m == 3 * NRB

    mod_a = jnp.dot(sc_s[...], wm_v[:, 0:2 * D], preferred_element_type=F32)
    h1 = xn * (1.0 + mod_a[:, D:2 * D]) + mod_a[:, 0:D]
    h_s[...] = h1.astype(BF16)

    def q_prep():
        whole(wq_v, wsem.at[6]).wait()
        q = jnp.dot(h_s[...], wq_v[...], preferred_element_type=F32)
        q = q[0:1, :] * (DH ** -0.5)
        for b in range(PAIR // 128):
            qb_s[b * 128:(b + 1) * 128, :] = jnp.broadcast_to(
                q[:, b * 128:(b + 1) * 128], (128, 128)).T

    q_prep()

    def head(h, carry):
        par = lax.rem(h, 2)

        def inject(t):
            for kd, n in slots.get(t, []):
                if kd == 'wq':
                    m = par * NWQ + n
                    tile = lax.div(m, NRB)
                    rows = pl.ds(pl.multiple_of(lax.rem(m, NRB) * WQR, 16), WQR)

                    @pl.when(h < H - 2)
                    def _():
                        col = pl.multiple_of((lax.div(h, 2) + 1) * PAIR + tile * 128, 128)
                        pltpu.make_async_copy(
                            wq_hbm.at[rows, pl.ds(col, 128)],
                            wq_v.at[rows, pl.ds(pl.multiple_of(tile * 128, 128), 128)],
                            wsem.at[6]).start(priority=HI)

                    @pl.when(h >= H - 2)
                    def _():
                        cols = pl.ds(pl.multiple_of(tile * 512, 128), 512)
                        pltpu.make_async_copy(
                            w1_hbm.at[rows, cols], w1_v.at[rows, cols],
                            wsem.at[9]).start(priority=HI)
                elif kd == 'wo':
                    pltpu.make_async_copy(
                        wo_hbm.at[pl.ds(pl.multiple_of(h * DH + n * 16, 16), 16), :],
                        wo_v.at[pl.ds(n * 16, 16), :], wsem.at[7]).start(priority=HI)
                else:
                    m = h * NWM + n

                    @pl.when(m < WM_TOT)
                    def _():
                        rows = pl.ds(pl.multiple_of(lax.rem(m, 40) * 16, 16), 16)
                        cols = pl.ds(pl.multiple_of((2 + lax.div(m, 40)) * D, 128), D)
                        pltpu.make_async_copy(
                            wm_hbm.at[rows, cols], wm_v.at[rows, cols],
                            wsem.at[5]).start(priority=HI)

                    if W2_EARLY:
                        @pl.when(jnp.logical_and(h >= WM_HEADS, m - WM_HEADS * NWM < W2_EARLY))
                        def _():
                            rows = pl.ds(pl.multiple_of((m - WM_HEADS * NWM) * 16, 16), 16)
                            pltpu.make_async_copy(
                                w2_hbm.at[rows, :], w2_v.at[rows, :],
                                wsem.at[8]).start(priority=HI)

        qb = qb_s[pl.ds(pl.multiple_of(par * DH, 16), DH), :]
        mx = None
        for j in range(NP):
            k_copy(h, j).wait()
            v_copy(h, j).start(priority=LO)
            inject(j)
            pr = kbuf[j].astype(F32) * qb
            s8 = _tree_sum(pr[i * 8:(i + 1) * 8] for i in range(DH // 8))
            s = jnp.broadcast_to(jnp.sum(s8, axis=0, keepdims=True), (8, TN))
            s_s[j] = s
            mx = s if mx is None else jnp.maximum(mx, s)
        m = jnp.max(mx, axis=1, keepdims=True)

        acc = None
        for j in range(NP):
            v_copy(h, j).wait()

            @pl.when(h < H - 1)
            def _():
                k_copy(h + 1, j).start(priority=LO)

            if tail[j]:
                @pl.when(h == H - 1)
                def _():
                    w2_tail(j).start(priority=LO)
            inject(NP + j)
            p = jnp.exp(s_s[j] - m)
            vt = vbuf[j].astype(F32)
            upd = [vt[i * 8:(i + 1) * 8] * p for i in range(DH // 8)] + [p]
            acc = upd if acc is None else [a + u for a, u in zip(acc, upd)]

        whole(wo_v, wsem.at[7]).wait()
        inv_l = 1.0 / jnp.sum(acc[-1], axis=1, keepdims=True)
        wo = wo_v[...].astype(F32)
        a = _tree_sum(wo[i * 8:(i + 1) * 8] * jnp.sum(acc[i], axis=1, keepdims=True)
                      for i in range(DH // 8))
        acc_s[...] += a * inv_l

        @pl.when(jnp.logical_and(par == 1, h < H - 1))
        def _():
            q_prep()

        @pl.when(h == WM_HEADS)
        def _():
            whole(wm_v.at[:, pl.ds(2 * D, 4 * D)], wsem.at[5]).wait()
            mod_s[...] = jnp.dot(sc_s[...], wm_v[:, 2 * D:6 * D],
                                 preferred_element_type=F32)

        return carry

    assert WM_HEADS < H
    lax.fori_loop(0, H, head, 0)

    cp_b1.wait()
    whole(w1_v, wsem.at[9]).wait()
    if W2_EARLY:
        whole(w2_v.at[pl.ds(0, W2_EARLY * 16), :], wsem.at[8]).wait()
    attn = jnp.sum(acc_s[...], axis=0, keepdims=True)
    x1 = x_v[0].astype(F32) + mod_s[0:1, 0:D] * attn
    h2 = _layernorm(x1) * (1.0 + mod_s[0:1, 2 * D:3 * D]) + mod_s[0:1, D:2 * D]
    h2 = jnp.broadcast_to(h2, (8, D)).astype(BF16)
    u = jnp.dot(h2, w1_v[...], preferred_element_type=F32)
    u = u + b1_v[...].astype(F32).reshape(1, FF)
    sp = jnp.log1p(jnp.exp(-jnp.abs(u))) + jnp.where(u > 0, u, 0.0)
    act32 = u * jnp.tanh(sp)
    act = act32.astype(BF16)
    nvb = cfg['vputail']
    for b in range(nvb):
        c0 = FF - (nvb - b) * 128
        ab_s[b * 128:(b + 1) * 128, :] = jnp.broadcast_to(
            act32[0:1, c0:c0 + 128], (128, 128)).T
    y = jnp.zeros((8, D), F32)
    blk = 0
    waited = 0

    def wait_upto(need):
        nonlocal waited
        while waited < NP and (tail[waited] == 0 or tail_off[waited] < need):
            if tail[waited]:
                w2_tail(waited).wait()
            waited += 1

    for g in cfg['tailg']:
        wait_upto((blk + g) * 8)
        y = y + jnp.dot(act[:, blk * 128:(blk + g) * 128],
                        w2_v[blk * 128:(blk + g) * 128, :],
                        preferred_element_type=F32)
        blk += g
    assert blk == FF // 128 - nvb
    y = y[0:1]
    if nvb:
        yv = jnp.zeros((8, D), F32)
        g0 = blk * 8
        done = g0
        while done < W2_G:
            wait_upto(done + 1)
            landed = min(W2_G, tail_off[waited] if waited < NP and tail[waited] else W2_G)
            for gi in range(done, landed):
                w = w2_v[gi * 16:(gi + 1) * 16, :].astype(F32)
                ab = ab_s[(gi - g0) * 16:(gi - g0 + 1) * 16, :]
                ab = jnp.concatenate([ab] * (D // 128), axis=1)
                pr = w * ab
                yv = yv + pr[0:8] + pr[8:16]
            done = landed
        y = y + jnp.sum(yv, axis=0, keepdims=True)
    wait_upto(10 ** 9)
    out = x1 + mod_s[0:1, 3 * D:4 * D] * y
    o_ref[0] = out.astype(o_ref.dtype)


def build(cfg):
    @jax.jit
    def fn(A_x, A_k_cache, A_v_cache, A_wq, A_wo, B_x, B_w1, B_b1, B_w2, c, w_mod):
        del B_x
        sk = A_k_cache.shape[2]
        win = min(4096, max(256, sk // 4))
        npc = win // TN
        kt = jnp.swapaxes(A_k_cache, 2, 3)
        vt = jnp.swapaxes(A_v_cache, 2, 3)
        any_spec = pl.BlockSpec(memory_space=pl.ANY)
        return pl.pallas_call(
            functools.partial(_kernel, win=win, start=sk - win, cfg=cfg),
            out_shape=jax.ShapeDtypeStruct((1, 1, D), A_x.dtype),
            in_specs=[any_spec] * 10,
            out_specs=pl.BlockSpec(memory_space=pltpu.VMEM),
            scratch_shapes=[
                pltpu.VMEM((1, 1, D), BF16),
                pltpu.VMEM((1, D), BF16),
                pltpu.VMEM((FF,), BF16),
                pltpu.VMEM((npc, DH, TN), BF16),
                pltpu.VMEM((npc, DH, TN), BF16),
                pltpu.VMEM((D, PAIR), BF16),
                pltpu.VMEM((DH, D), BF16),
                pltpu.VMEM((D, FF), BF16),
                pltpu.VMEM((FF, D), BF16),
                pltpu.VMEM((D, 6 * D), BF16),
                pltpu.VMEM((8, D), BF16),
                pltpu.VMEM((8, D), BF16),
                pltpu.VMEM((PAIR, 128), F32),
                pltpu.VMEM((npc, 8, TN), F32),
                pltpu.VMEM((8, D), F32),
                pltpu.VMEM((8, 4 * D), F32),
                pltpu.VMEM((256, 128), F32),
                pltpu.SemaphoreType.DMA((npc,)),
                pltpu.SemaphoreType.DMA((D // 16,)),
                pltpu.SemaphoreType.DMA((10,)),
            ],
            compiler_params=pltpu.CompilerParams(vmem_limit_bytes=64 * 1024 * 1024,
                                                 disable_bounds_checks=True,
                                                 disable_semaphore_checks=True),
            name="adaln_decode",
        )(A_x, c, B_b1, kt, vt, A_wq, A_wo, B_w1, B_w2, w_mod)
    return fn

pallas_adaLN_cond__sliding_block_cached__dense_activation_mish__decode_kernel = build(CFG)
```

```python
import functools

import jax
import jax.numpy as jnp
from jax import lax
import jax.experimental.pallas as pl
import jax.experimental.pallas.tpu as pltpu

F32 = jnp.float32
BF16 = jnp.bfloat16

D = 640
H = 32
DH = 192
FF = 1536
EPS = 1e-5
PAIR = 2 * DH
LO, HI = 1, 0
TN = 128
RG = 8
HD = D // 2
NWQ = HD // RG // 2
WQ_AHEAD = 9
WO_COLS = ((0, 256), (256, 256), (512, 128))
NWO = (DH // RG) * len(WO_COLS)
NWM = 12
WM_TOT = (D // RG) * 4
WM_HEADS = -(-WM_TOT // NWM)
NA = D // 16
NL0 = 24
Q_TICKS = (8, 11, 14, 17)
WO_TICKS = (6, 10, 14)
MOD_TICKS = (18, 22, 26, 30)
W2_MXU = (4, 4, 2)
W2_VPU = FF // 128 - sum(W2_MXU)
W2_ROWS = 48
S_X, S_C, S_B1, S_WM, S_W1 = 0, 1, 2, 3, 4
S_WQ, S_WO = 5, 7


def _layernorm(x):
    m = jnp.mean(x, axis=-1, keepdims=True)
    xc = x - m
    v = jnp.mean(xc * xc, axis=-1, keepdims=True)
    return xc / jnp.sqrt(v + EPS)


def _tree_sum(xs):
    xs = list(xs)
    while len(xs) > 1:
        xs = [xs[i] + xs[i + 1] if i + 1 < len(xs) else xs[i]
              for i in range(0, len(xs), 2)]
    return xs[0]


def _lane_bcast(row):
    return jnp.broadcast_to(row, (128, 128)).T


def _kernel(x_hbm, c_hbm, b1_hbm, k_hbm, v_hbm, wq_hbm, wo_hbm, w1_hbm, w2_hbm,
            wm_hbm, o_ref,
            x_v, c_v, b1_v, kbuf, vbuf, wq_v, wo_v, w1_v, w2_v, wm_v,
            h_s, sc_s, q_s, qb_s, s_s, av_s, acc_s, mod_s, ab_s,
            ksem, vsem, psem, wsem, *, win, start):
    nt = win // TN
    assert nt * W2_ROWS == FF

    def k_copy(h, j):
        return pltpu.make_async_copy(
            k_hbm.at[0, h, :, pl.ds(start + j * TN, TN)], kbuf.at[j], ksem.at[j])

    def v_copy(h, j):
        return pltpu.make_async_copy(
            v_hbm.at[0, h, :, pl.ds(start + j * TN, TN)], vbuf.at[j], vsem.at[j])

    def w2_copy(j):
        rows = pl.ds(j * W2_ROWS, W2_ROWS)
        return pltpu.make_async_copy(w2_hbm.at[rows, :], w2_v.at[rows, :], ksem.at[j])

    def wq_copy(pair, rows):
        col = pair * PAIR
        slot = pair % 2
        if not isinstance(pair, int):
            col = pl.multiple_of(col, 128)
        return pltpu.make_async_copy(
            wq_hbm.at[:, rows, pl.ds(col, PAIR)], wq_v.at[slot, :, rows, :],
            wsem.at[S_WQ + slot])

    def wait_all(ref, sem):
        pltpu.make_async_copy(ref, ref, sem).wait()

    items = sorted(((i + 0.5) / n, kind, i)
                   for kind, n in (("wq", NWQ), ("wo", NWO), ("wm", NWM))
                   for i in range(n))
    slots = {}
    for i, (_, kind, n) in enumerate(items):
        slots.setdefault((i * (2 * nt - 1)) // len(items), []).append((kind, n))

    cp_x = pltpu.make_async_copy(x_hbm, x_v, wsem.at[S_X])
    cp_c = pltpu.make_async_copy(c_hbm, c_v, wsem.at[S_C])
    cp_b1 = pltpu.make_async_copy(b1_hbm, b1_v, wsem.at[S_B1])

    def wma_copy(i):
        rows, cols = pl.ds(i * 16, 16), pl.ds(0, 2 * D)
        return pltpu.make_async_copy(
            wm_hbm.at[rows, cols], wm_v.at[rows, cols], psem.at[i])

    lows = [wma_copy(i) for i in range(NA)] + [k_copy(0, j) for j in range(nt)]
    for i in range(NL0):
        lows[i].start(priority=LO)
        if i % 8 == 7:
            (cp_c, cp_x, cp_b1)[i // 8].start(priority=HI)
    n_lo, n_hi, tot_hi = NL0, 0, 2 * NWQ + WQ_AHEAD
    for i in range(NA):
        lows[i].wait()
        ahead = NL0 + max(0, (i + 1 - (NA - NL0)) * (nt - NL0) // NL0)
        while n_lo < i + 1 + ahead:
            lows[n_lo].start(priority=LO)
            n_lo += 1
        while n_hi < min(tot_hi, ((i + 1) * tot_hi) // (NA - 2)):
            pair, rb = divmod(n_hi, 2 * NWQ)
            wq_copy(pair, pl.ds(rb * RG, RG)).start(priority=HI)
            n_hi += 1
        if i == 8:
            acc_s[...] = jnp.zeros_like(acc_s)
            cp_c.wait()
            cp_x.wait()
            c = c_v[...].astype(F32)
            sc = c * (1.0 / (1.0 + jnp.exp(-c)))
            sc_s[...] = jnp.broadcast_to(sc, sc_s.shape).astype(BF16)
            xn = _layernorm(x_v[0].astype(F32))
    assert n_lo == len(lows) and n_hi == tot_hi

    mod_a = jnp.dot(sc_s[...], wm_v[:, 0:2 * D], preferred_element_type=F32)
    h_s[...] = (xn * (1.0 + mod_a[:, D:2 * D]) + mod_a[:, 0:D]).astype(BF16)

    def q_dot(slot):
        wait_all(wq_v.at[slot], wsem.at[S_WQ + slot])
        q = jnp.dot(h_s[...], wq_v[slot].reshape(D, PAIR), preferred_element_type=F32)
        q_s[...] = q * (DH ** -0.5)

    def q_bcast(b):
        qb_s[b * 128:(b + 1) * 128, :] = _lane_bcast(q_s[0:1, b * 128:(b + 1) * 128])

    q_dot(0)
    for b in range(PAIR // 128):
        q_bcast(b)

    def wo_apply(slot, g0, g1):
        if g0 == 0:
            wait_all(wo_v.at[slot], wsem.at[S_WO + slot])
        inv_l = 1.0 / jnp.sum(av_s[DH:DH + 8, :], axis=1, keepdims=True)
        wo = wo_v[slot, g0 * 8:g1 * 8, :].astype(F32)
        a = _tree_sum(
            wo[(g - g0) * 8:(g - g0 + 1) * 8]
            * jnp.sum(av_s[g * 8:(g + 1) * 8, :], axis=1, keepdims=True)
            for g in range(g0, g1))
        acc_s[...] += a * inv_l

    def head(h, carry):
        par = lax.rem(h, 2)

        def inject(t):
            for kind, n in slots.get(t, []):
                if kind == "wq":
                    g = h * NWQ + (n + WQ_AHEAD)
                    prev = lax.div(g, 2 * NWQ)
                    rows = pl.ds(pl.multiple_of((g - prev * (2 * NWQ)) * RG, RG), RG)

                    @pl.when(prev < H // 2 - 1)
                    def _():
                        wq_copy(prev + 1, rows).start(priority=HI)

                    @pl.when(prev == H // 2 - 1)
                    def _():
                        pltpu.make_async_copy(
                            w1_hbm.at[:, rows, :], w1_v.at[:, rows, :],
                            wsem.at[S_W1]).start(priority=HI)
                elif kind == "wo":
                    rg, ci = divmod(n, len(WO_COLS))
                    cols = pl.ds(*WO_COLS[ci])
                    pltpu.make_async_copy(
                        wo_hbm.at[pl.ds(pl.multiple_of(h * DH + rg * RG, RG), RG), cols],
                        wo_v.at[par, pl.ds(rg * RG, RG), cols],
                        wsem.at[S_WO + par]).start(priority=HI)
                else:
                    m = h * NWM + n

                    @pl.when(m < WM_TOT)
                    def _():
                        rows = pl.ds(pl.multiple_of(lax.div(m, 4) * RG, RG), RG)
                        cols = pl.ds(pl.multiple_of((2 + lax.rem(m, 4)) * D, 128), D)
                        pltpu.make_async_copy(
                            wm_hbm.at[rows, cols], wm_v.at[rows, cols],
                            wsem.at[S_WM]).start(priority=HI)

        qb = qb_s[pl.ds(pl.multiple_of(par * DH, 8), DH), :]
        mx = None
        for j in range(nt):
            k_copy(h, j).wait()
            v_copy(h, j).start(priority=LO)
            inject(j)
            pr = kbuf[j].astype(F32) * qb
            s8 = _tree_sum(pr[i * 8:(i + 1) * 8] for i in range(DH // 8))
            s = jnp.broadcast_to(jnp.sum(s8, axis=0, keepdims=True), (8, TN))
            s_s[j] = s
            mx = s if mx is None else jnp.maximum(mx, s)
            if j in WO_TICKS:
                ng = DH // 8 // len(WO_TICKS)
                g0 = WO_TICKS.index(j) * ng

                @pl.when(h > 0)
                def _():
                    wo_apply(1 - par, g0, g0 + ng)
            if j in MOD_TICKS:
                g = MOD_TICKS.index(j)

                @pl.when(h == WM_HEADS)
                def _():
                    if g == 0:
                        wait_all(wm_v.at[:, pl.ds(2 * D, 4 * D)], wsem.at[S_WM])
                    mod_s[:, g * D:(g + 1) * D] = jnp.dot(
                        sc_s[...], wm_v[:, (2 + g) * D:(3 + g) * D],
                        preferred_element_type=F32)
        row_max = jnp.max(mx, axis=1, keepdims=True)

        acc = None
        for j in range(nt):
            v_copy(h, j).wait()

            @pl.when(h < H - 1)
            def _():
                k_copy(h + 1, j).start(priority=LO)

            @pl.when(h == H - 1)
            def _():
                w2_copy(j).start(priority=LO)

            inject(nt + j)
            p = jnp.exp(s_s[j] - row_max)
            vt = vbuf[j].astype(F32)
            upd = [vt[i * 8:(i + 1) * 8] * p for i in range(DH // 8)] + [p]
            acc = upd if acc is None else [a + u for a, u in zip(acc, upd)]
            if j in Q_TICKS:
                g = Q_TICKS.index(j)

                @pl.when(jnp.logical_and(par == 1, h < H - 1))
                def _():
                    if g == 0:
                        q_dot(lax.rem(lax.div(h, 2) + 1, 2))
                    else:
                        q_bcast(g - 1)
        for i in range(DH // 8 + 1):
            av_s[i * 8:(i + 1) * 8, :] = acc[i]
        return carry

    lax.fori_loop(0, H, head, 0)

    cp_b1.wait()
    wait_all(w1_v, wsem.at[S_W1])
    wo_apply((H - 1) % 2, 0, DH // 8)
    attn = jnp.sum(acc_s[...], axis=0, keepdims=True)
    x1 = x_v[0].astype(F32) + mod_s[0:1, 0:D] * attn
    h2 = _layernorm(x1) * (1.0 + mod_s[0:1, 2 * D:3 * D]) + mod_s[0:1, D:2 * D]
    h2 = jnp.broadcast_to(h2, (8, D)).astype(BF16)
    u = jnp.dot(h2, w1_v[...].reshape(D, FF), preferred_element_type=F32)
    u = u + b1_v[...].astype(F32).reshape(1, FF)
    sp = jnp.log1p(jnp.exp(-jnp.abs(u))) + jnp.where(u > 0, u, 0.0)
    act32 = u * jnp.tanh(sp)
    act = act32.astype(BF16)
    r_vpu = FF - W2_VPU * 128
    for b in range(W2_VPU):
        ab_s[b * 128:(b + 1) * 128, :] = _lane_bcast(
            act32[0:1, r_vpu + b * 128:r_vpu + (b + 1) * 128])

    y = jnp.zeros((8, D), F32)
    r0 = waited = 0
    for g in W2_MXU:
        r1 = r0 + g * 128
        while waited * W2_ROWS < r1:
            w2_copy(waited).wait()
            waited += 1
        y = y + jnp.dot(act[:, r0:r1], w2_v[r0:r1, :], preferred_element_type=F32)
        r0 = r1
    yv = jnp.zeros((8, D), F32)
    while r0 < FF:
        if waited * W2_ROWS <= r0:
            w2_copy(waited).wait()
            waited += 1
        for r in range(r0, waited * W2_ROWS, 16):
            ab = ab_s[r - r_vpu:r - r_vpu + 16, :]
            pr = w2_v[r:r + 16, :].astype(F32) * jnp.concatenate([ab] * (D // 128), axis=1)
            yv = yv + pr[0:8] + pr[8:16]
        r0 = waited * W2_ROWS
    y = y[0:1] + jnp.sum(yv, axis=0, keepdims=True)
    o_ref[0] = (x1 + mod_s[0:1, 3 * D:4 * D] * y).astype(o_ref.dtype)


@jax.jit
def pallas_adaLN_cond__sliding_block_cached__dense_activation_mish__decode_kernel(
    A_x: jax.Array,
    A_k_cache: jax.Array,
    A_v_cache: jax.Array,
    A_wq: jax.Array,
    A_wo: jax.Array,
    B_x: jax.Array,
    B_w1: jax.Array,
    B_b1: jax.Array,
    B_w2: jax.Array,
    c: jax.Array,
    w_mod: jax.Array,
):
    del B_x
    sk = A_k_cache.shape[2]
    win = min(4096, max(256, sk // 4))
    assert A_x.shape == (1, 1, D) and A_k_cache.shape == (1, H, sk, DH)
    assert (sk - win) % TN == 0
    nt = win // TN
    return pl.pallas_call(
        functools.partial(_kernel, win=win, start=sk - win),
        out_shape=jax.ShapeDtypeStruct((1, 1, D), A_x.dtype),
        in_specs=[pl.BlockSpec(memory_space=pl.ANY)] * 10,
        out_specs=pl.BlockSpec(memory_space=pltpu.VMEM),
        scratch_shapes=[
            pltpu.VMEM((1, 1, D), BF16),
            pltpu.VMEM((1, D), BF16),
            pltpu.VMEM((FF,), BF16),
            pltpu.VMEM((nt, DH, TN), BF16),
            pltpu.VMEM((nt, DH, TN), BF16),
            pltpu.VMEM((2, 2, HD, PAIR), BF16),
            pltpu.VMEM((2, DH, D), BF16),
            pltpu.VMEM((2, HD, FF), BF16),
            pltpu.VMEM((FF, D), BF16),
            pltpu.VMEM((D, 6 * D), BF16),
            pltpu.VMEM((8, D), BF16),
            pltpu.VMEM((8, D), BF16),
            pltpu.VMEM((8, PAIR), F32),
            pltpu.VMEM((PAIR, 128), F32),
            pltpu.VMEM((nt, 8, TN), F32),
            pltpu.VMEM((DH + 8, 128), F32),
            pltpu.VMEM((8, D), F32),
            pltpu.VMEM((8, 4 * D), F32),
            pltpu.VMEM((W2_VPU * 128, 128), F32),
            pltpu.SemaphoreType.DMA((nt,)),
            pltpu.SemaphoreType.DMA((nt,)),
            pltpu.SemaphoreType.DMA((NA,)),
            pltpu.SemaphoreType.DMA((9,)),
        ],
        compiler_params=pltpu.CompilerParams(
            vmem_limit_bytes=64 * 1024 * 1024,
            disable_bounds_checks=True,
            disable_semaphore_checks=True),
        name="adaln_decode",
    )(A_x, c, B_b1,
      jnp.swapaxes(A_k_cache, 2, 3), jnp.swapaxes(A_v_cache, 2, 3),
      A_wq.reshape(2, HD, H * DH), A_wo, B_w1.reshape(2, HD, FF), B_w2, w_mod)
```

```python
import functools

import jax
import jax.numpy as jnp
from jax import lax
import jax.experimental.pallas as pl
import jax.experimental.pallas.tpu as pltpu

F32 = jnp.float32
BF16 = jnp.bfloat16

D = 640
H = 32
DH = 192
FF = 1536
EPS = 1e-5
GH = 4
GC = GH * DH
LO, HI = 1, 0
TN = 128
RG = 8
HD = D // 2
NG = HD // RG
NWQ = NG // GH
WQ_AHEAD = 5
KM = 10
MR = D // KM
WO_COLS = ((0, 256), (256, 256), (512, 128))
NWO = (DH // RG) * len(WO_COLS)
NWM = 11
WM_TOT = (D // RG) * 4
WM_HEADS = -(-WM_TOT // NWM)
PW = 256
NA = (MR // RG) * (2 * D // PW)
NL0 = 24
Q_TICKS = (8, 11, 14, 17, 20, 23, 26)
WO_TICKS = (6, 10, 14)
MOD_TICKS = (18, 22, 26, 30)
W2_MXU = (4, 4, 2)
W2_VPU = FF // 128 - sum(W2_MXU)
W2_ROWS = 48
S_X, S_C, S_B1, S_WM, S_W1 = 0, 1, 2, 3, 4
S_WQ, S_WO = 5, 7


def _layernorm(x):
    m = jnp.mean(x, axis=-1, keepdims=True)
    xc = x - m
    v = jnp.mean(xc * xc, axis=-1, keepdims=True)
    return xc / jnp.sqrt(v + EPS)


def _tree_sum(xs):
    xs = list(xs)
    while len(xs) > 1:
        xs = [xs[i] + xs[i + 1] if i + 1 < len(xs) else xs[i]
              for i in range(0, len(xs), 2)]
    return xs[0]


def _lane_bcast(row):
    return jnp.broadcast_to(row, (128, 128)).T


def _kernel(x_hbm, c_hbm, b1_hbm, k_hbm, v_hbm, wq_hbm, wo_hbm, w1_hbm, w2_hbm,
            wm_hbm, o_ref,
            x_v, c_v, b1_v, kbuf, vbuf, wq_v, wo_v, w1_v, w2_v, wm_v,
            h_s, sc_s, q_s, qb_s, s_s, av_s, acc_s, mod_s, ab_s,
            ksem, vsem, psem, wsem, *, win, start):
    nt = win // TN
    assert nt * W2_ROWS == FF

    def k_copy(h, j):
        return pltpu.make_async_copy(
            k_hbm.at[0, h, :, pl.ds(start + j * TN, TN)], kbuf.at[j], ksem.at[j])

    def v_copy(h, j):
        return pltpu.make_async_copy(
            v_hbm.at[0, h, :, pl.ds(start + j * TN, TN)], vbuf.at[j], vsem.at[j])

    def w2_copy(j):
        rows = pl.ds(j * W2_ROWS, W2_ROWS)
        return pltpu.make_async_copy(w2_hbm.at[rows, :], w2_v.at[rows, :], ksem.at[j])

    def wq_copy(grp, rows):
        if isinstance(grp, int):
            col, slot = grp * GC, grp % 2
        else:
            col, slot = pl.multiple_of(grp * GC, 128), lax.rem(grp, 2)
        return pltpu.make_async_copy(
            wq_hbm.at[:, rows, pl.ds(col, GC)], wq_v.at[slot, :, rows, :],
            wsem.at[S_WQ + slot])

    def wait_all(ref, sem):
        pltpu.make_async_copy(ref, ref, sem).wait()

    items = sorted(((i + 0.5) / n, kind, i)
                   for kind, n in (("wq", NWQ), ("wo", NWO), ("wm", NWM))
                   for i in range(n))
    slots = {}
    for i, (_, kind, n) in enumerate(items):
        slots.setdefault((i * (2 * nt - 1)) // len(items), []).append((kind, n))

    cp_x = pltpu.make_async_copy(x_hbm, x_v, wsem.at[S_X])
    cp_c = pltpu.make_async_copy(c_hbm, c_v, wsem.at[S_C])
    cp_b1 = pltpu.make_async_copy(b1_hbm, b1_v, wsem.at[S_B1])

    def wma_copy(i):
        rb, cb = divmod(i, 2 * D // PW)
        rows, cols = pl.ds(rb * RG, RG), pl.ds(cb * PW, PW)
        return pltpu.make_async_copy(
            wm_hbm.at[:, rows, cols], wm_v.at[:, rows, cols], psem.at[i])

    lows = [wma_copy(i) for i in range(NA)] + [k_copy(0, j) for j in range(nt)]
    for i in range(NL0):
        lows[i].start(priority=LO)
        if i % 8 == 7:
            (cp_c, cp_x, cp_b1)[i // 8].start(priority=HI)
    n_lo, n_hi, tot_hi = NL0, 0, NG + WQ_AHEAD
    for i in range(NA):
        lows[i].wait()
        ahead = NL0 + max(0, (i + 1 - (NA - NL0)) * (nt - NL0) // NL0)
        while n_lo < i + 1 + ahead:
            lows[n_lo].start(priority=LO)
            n_lo += 1
        while n_hi < min(tot_hi, ((i + 1) * tot_hi) // (NA - 2)):
            grp, rb = divmod(n_hi, NG)
            wq_copy(grp, pl.ds(rb * RG, RG)).start(priority=HI)
            n_hi += 1
        if i == 8:
            acc_s[...] = jnp.zeros_like(acc_s)
            cp_c.wait()
            cp_x.wait()
            c = c_v[...].astype(F32)
            sc = c * (1.0 / (1.0 + jnp.exp(-c)))
            sc_s[...] = jnp.broadcast_to(sc, sc_s.shape).astype(BF16)
            xn = _layernorm(x_v[0].astype(F32))
    assert n_lo == len(lows) and n_hi == tot_hi

    mod_a = jnp.dot(sc_s[...], wm_v[:, :, 0:2 * D].reshape(D, 2 * D),
                    preferred_element_type=F32)
    h_s[...] = (xn * (1.0 + mod_a[:, D:2 * D]) + mod_a[:, 0:D]).astype(BF16)

    def q_dot(slot):
        wait_all(wq_v.at[slot], wsem.at[S_WQ + slot])
        q = jnp.dot(h_s[...], wq_v[slot].reshape(D, GC), preferred_element_type=F32)
        q_s[...] = q * (DH ** -0.5)

    def q_bcast(b):
        qb_s[b * 128:(b + 1) * 128, :] = _lane_bcast(q_s[0:1, b * 128:(b + 1) * 128])

    q_dot(0)
    for b in range(GC // 128):
        q_bcast(b)

    def wo_apply(slot, g0, g1):
        if g0 == 0:
            wait_all(wo_v.at[slot], wsem.at[S_WO + slot])
        inv_l = 1.0 / jnp.sum(av_s[DH:DH + 8, :], axis=1, keepdims=True)
        wo = wo_v[slot, g0 * 8:g1 * 8, :].astype(F32)
        a = _tree_sum(
            wo[(g - g0) * 8:(g - g0 + 1) * 8]
            * jnp.sum(av_s[g * 8:(g + 1) * 8, :], axis=1, keepdims=True)
            for g in range(g0, g1))
        acc_s[...] += a * inv_l

    def head(h, carry):
        par = lax.rem(h, 2)

        def inject(t):
            for kind, n in slots.get(t, []):
                if kind == "wq":
                    g = h * NWQ + (n + WQ_AHEAD)
                    prev = lax.div(g, NG)
                    rows = pl.ds(pl.multiple_of((g - prev * NG) * RG, RG), RG)

                    @pl.when(prev < H // GH - 1)
                    def _():
                        wq_copy(prev + 1, rows).start(priority=HI)

                    @pl.when(prev == H // GH - 1)
                    def _():
                        pltpu.make_async_copy(
                            w1_hbm.at[:, rows, :], w1_v.at[:, rows, :],
                            wsem.at[S_W1]).start(priority=HI)
                elif kind == "wo":
                    rg, ci = divmod(n, len(WO_COLS))
                    cols = pl.ds(*WO_COLS[ci])
                    pltpu.make_async_copy(
                        wo_hbm.at[pl.ds(pl.multiple_of(h * DH + rg * RG, RG), RG), cols],
                        wo_v.at[par, pl.ds(rg * RG, RG), cols],
                        wsem.at[S_WO + par]).start(priority=HI)
                else:
                    m = h * NWM + n

                    @pl.when(m < WM_TOT)
                    def _():
                        rb = lax.div(m, 4)
                        k = lax.div(rb, MR // RG)
                        rows = pl.ds(pl.multiple_of((rb - k * (MR // RG)) * RG, RG), RG)
                        cols = pl.ds(pl.multiple_of((2 + lax.rem(m, 4)) * D, 128), D)
                        pltpu.make_async_copy(
                            wm_hbm.at[k, rows, cols], wm_v.at[k, rows, cols],
                            wsem.at[S_WM]).start(priority=HI)

        qb = qb_s[pl.ds(pl.multiple_of(lax.rem(h, GH) * DH, 8), DH), :]
        mx = None
        for j in range(nt):
            k_copy(h, j).wait()
            v_copy(h, j).start(priority=LO)
            inject(j)
            pr = kbuf[j].astype(F32) * qb
            s8 = _tree_sum(pr[i * 8:(i + 1) * 8] for i in range(DH // 8))
            s = jnp.broadcast_to(jnp.sum(s8, axis=0, keepdims=True), (8, TN))
            s_s[j] = s
            mx = s if mx is None else jnp.maximum(mx, s)
            if j in WO_TICKS:
                ng = DH // 8 // len(WO_TICKS)
                g0 = WO_TICKS.index(j) * ng

                @pl.when(h > 0)
                def _():
                    wo_apply(1 - par, g0, g0 + ng)
            if j in MOD_TICKS:
                g = MOD_TICKS.index(j)

                @pl.when(h == WM_HEADS)
                def _():
                    if g == 0:
                        wait_all(wm_v.at[:, :, pl.ds(2 * D, 4 * D)], wsem.at[S_WM])
                    mod_s[:, g * D:(g + 1) * D] = jnp.dot(
                        sc_s[...], wm_v[:, :, (2 + g) * D:(3 + g) * D].reshape(D, D),
                        preferred_element_type=F32)
        row_max = jnp.max(mx, axis=1, keepdims=True)

        acc = None
        for j in range(nt):
            v_copy(h, j).wait()

            @pl.when(h < H - 1)
            def _():
                k_copy(h + 1, j).start(priority=LO)

            @pl.when(h == H - 1)
            def _():
                w2_copy(j).start(priority=LO)

            inject(nt + j)
            p = jnp.exp(s_s[j] - row_max)
            vt = vbuf[j].astype(F32)
            upd = [vt[i * 8:(i + 1) * 8] * p for i in range(DH // 8)] + [p]
            acc = upd if acc is None else [a + u for a, u in zip(acc, upd)]
            if j in Q_TICKS:
                g = Q_TICKS.index(j)

                @pl.when(jnp.logical_and(lax.rem(h, GH) == GH - 1, h < H - 1))
                def _():
                    if g == 0:
                        q_dot(lax.rem(lax.div(h, GH) + 1, 2))
                    else:
                        q_bcast(g - 1)
        for i in range(DH // 8 + 1):
            av_s[i * 8:(i + 1) * 8, :] = acc[i]
        return carry

    lax.fori_loop(0, H, head, 0)

    cp_b1.wait()
    wait_all(w1_v, wsem.at[S_W1])
    wo_apply((H - 1) % 2, 0, DH // 8)
    attn = jnp.sum(acc_s[...], axis=0, keepdims=True)
    x1 = x_v[0].astype(F32) + mod_s[0:1, 0:D] * attn
    h2 = _layernorm(x1) * (1.0 + mod_s[0:1, 2 * D:3 * D]) + mod_s[0:1, D:2 * D]
    h2 = jnp.broadcast_to(h2, (8, D)).astype(BF16)
    u = jnp.dot(h2, w1_v[...].reshape(D, FF), preferred_element_type=F32)
    u = u + b1_v[...].astype(F32).reshape(1, FF)
    sp = jnp.log1p(jnp.exp(-jnp.abs(u))) + jnp.where(u > 0, u, 0.0)
    act32 = u * jnp.tanh(sp)
    act = act32.astype(BF16)
    r_vpu = FF - W2_VPU * 128
    for b in range(W2_VPU):
        ab_s[b * 128:(b + 1) * 128, :] = _lane_bcast(
            act32[0:1, r_vpu + b * 128:r_vpu + (b + 1) * 128])

    y = jnp.zeros((8, D), F32)
    r0 = waited = 0
    for g in W2_MXU:
        r1 = r0 + g * 128
        while waited * W2_ROWS < r1:
            w2_copy(waited).wait()
            waited += 1
        y = y + jnp.dot(act[:, r0:r1], w2_v[r0:r1, :], preferred_element_type=F32)
        r0 = r1
    yv = jnp.zeros((8, D), F32)
    while r0 < FF:
        if waited * W2_ROWS <= r0:
            w2_copy(waited).wait()
            waited += 1
        for r in range(r0, waited * W2_ROWS, 16):
            ab = ab_s[r - r_vpu:r - r_vpu + 16, :]
            pr = w2_v[r:r + 16, :].astype(F32) * jnp.concatenate([ab] * (D // 128), axis=1)
            yv = yv + pr[0:8] + pr[8:16]
        r0 = waited * W2_ROWS
    y = y[0:1] + jnp.sum(yv, axis=0, keepdims=True)
    o_ref[0] = (x1 + mod_s[0:1, 3 * D:4 * D] * y).astype(o_ref.dtype)


@jax.jit
def pallas_adaLN_cond__sliding_block_cached__dense_activation_mish__decode_kernel(
    A_x: jax.Array,
    A_k_cache: jax.Array,
    A_v_cache: jax.Array,
    A_wq: jax.Array,
    A_wo: jax.Array,
    B_x: jax.Array,
    B_w1: jax.Array,
    B_b1: jax.Array,
    B_w2: jax.Array,
    c: jax.Array,
    w_mod: jax.Array,
):
    del B_x
    sk = A_k_cache.shape[2]
    win = min(4096, max(256, sk // 4))
    assert A_x.shape == (1, 1, D) and A_k_cache.shape == (1, H, sk, DH)
    assert (sk - win) % TN == 0
    nt = win // TN
    return pl.pallas_call(
        functools.partial(_kernel, win=win, start=sk - win),
        out_shape=jax.ShapeDtypeStruct((1, 1, D), A_x.dtype),
        in_specs=[pl.BlockSpec(memory_space=pl.ANY)] * 10,
        out_specs=pl.BlockSpec(memory_space=pltpu.VMEM),
        scratch_shapes=[
            pltpu.VMEM((1, 1, D), BF16),
            pltpu.VMEM((1, D), BF16),
            pltpu.VMEM((FF,), BF16),
            pltpu.VMEM((nt, DH, TN), BF16),
            pltpu.VMEM((nt, DH, TN), BF16),
            pltpu.VMEM((2, 2, HD, GC), BF16),
            pltpu.VMEM((2, DH, D), BF16),
            pltpu.VMEM((2, HD, FF), BF16),
            pltpu.VMEM((FF, D), BF16),
            pltpu.VMEM((KM, MR, 6 * D), BF16),
            pltpu.VMEM((8, D), BF16),
            pltpu.VMEM((8, D), BF16),
            pltpu.VMEM((8, GC), F32),
            pltpu.VMEM((GC, 128), F32),
            pltpu.VMEM((nt, 8, TN), F32),
            pltpu.VMEM((DH + 8, 128), F32),
            pltpu.VMEM((8, D), F32),
            pltpu.VMEM((8, 4 * D), F32),
            pltpu.VMEM((W2_VPU * 128, 128), F32),
            pltpu.SemaphoreType.DMA((nt,)),
            pltpu.SemaphoreType.DMA((nt,)),
            pltpu.SemaphoreType.DMA((NA,)),
            pltpu.SemaphoreType.DMA((9,)),
        ],
        compiler_params=pltpu.CompilerParams(
            vmem_limit_bytes=64 * 1024 * 1024,
            disable_bounds_checks=True,
            disable_semaphore_checks=True),
        name="adaln_decode",
    )(A_x, c, B_b1,
      jnp.swapaxes(A_k_cache, 2, 3), jnp.swapaxes(A_v_cache, 2, 3),
      A_wq.reshape(2, HD, H * DH), A_wo, B_w1.reshape(2, HD, FF), B_w2,
      w_mod.reshape(KM, MR, 6 * D))
```

```python
import functools

import jax
import jax.numpy as jnp
from jax import lax
import jax.experimental.pallas as pl
import jax.experimental.pallas.tpu as pltpu

F32 = jnp.float32
BF16 = jnp.bfloat16

D = 640
H = 32
DH = 192
FF = 1536
EPS = 1e-5
GH = 4
GC = GH * DH
LO, HI = 1, 0
TN = 128
RG = 8
HD = D // 2
NG = HD // RG
NWQ = NG // GH
WQ_AHEAD = 5
KM = 10
MR = D // KM
WO_COLS = ((0, 256), (256, 256), (512, 128))
NWO = (DH // RG) * len(WO_COLS)
NWM = 11
WM_TOT = (D // RG) * 4
WM_HEADS = -(-WM_TOT // NWM)
PW = 256
NA = (MR // RG) * (2 * D // PW)
NL0 = 24
Q_TICKS = (8, 11, 14, 17, 20, 23, 26)
WO_TICKS = (6, 10, 14)
MOD_TICKS = (18, 22, 26, 30)
W2_MXU = (4, 4, 2)
W2_VPU = FF // 128 - sum(W2_MXU)
W2_ROWS = (48,) * 27 + (64, 64, 64, 32, 16)
W2_OFF = tuple(sum(W2_ROWS[:i]) for i in range(len(W2_ROWS) + 1))
S_X, S_C, S_B1, S_WM, S_W1 = 0, 1, 2, 3, 4
S_WQ, S_WO = 5, 7


def _layernorm(x):
    m = jnp.mean(x, axis=-1, keepdims=True)
    xc = x - m
    v = jnp.mean(xc * xc, axis=-1, keepdims=True)
    return xc / jnp.sqrt(v + EPS)


def _tree_sum(xs):
    xs = list(xs)
    while len(xs) > 1:
        xs = [xs[i] + xs[i + 1] if i + 1 < len(xs) else xs[i]
              for i in range(0, len(xs), 2)]
    return xs[0]


def _lane_bcast(row):
    return jnp.broadcast_to(row, (128, 128)).T


def _kernel(x_hbm, c_hbm, b1_hbm, k_hbm, v_hbm, wq_hbm, wo_hbm, w1_hbm, w2_hbm,
            wm_hbm, o_ref,
            x_v, c_v, b1_v, kbuf, vbuf, wq_v, wo_v, w1_v, w2_v, wm_v,
            h_s, sc_s, q_s, qb_s, s_s, av_s, acc_s, mod_s, ab_s,
            ksem, vsem, psem, wsem, *, win, start):
    nt = win // TN
    assert nt == len(W2_ROWS) and W2_OFF[-1] == FF

    def k_copy(h, j):
        return pltpu.make_async_copy(
            k_hbm.at[0, h, :, pl.ds(start + j * TN, TN)], kbuf.at[j], ksem.at[j])

    def v_copy(h, j):
        return pltpu.make_async_copy(
            v_hbm.at[0, h, :, pl.ds(start + j * TN, TN)], vbuf.at[j], vsem.at[j])

    def w2_copy(j):
        rows = pl.ds(W2_OFF[j], W2_ROWS[j])
        return pltpu.make_async_copy(w2_hbm.at[rows, :], w2_v.at[rows, :], ksem.at[j])

    def wq_copy(grp, rows, c0=0, width=GC):
        if isinstance(grp, int):
            col, slot = grp * GC + c0, grp % 2
        else:
            col, slot = pl.multiple_of(grp * GC + c0, 128), lax.rem(grp, 2)
        return pltpu.make_async_copy(
            wq_hbm.at[:, rows, pl.ds(col, width)],
            wq_v.at[slot, :, rows, pl.ds(c0, width)], wsem.at[S_WQ + slot])

    def wait_all(ref, sem):
        pltpu.make_async_copy(ref, ref, sem).wait()

    items = sorted(((i + 0.5) / n, kind, i)
                   for kind, n in (("wq", NWQ), ("wo", NWO), ("wm", NWM))
                   for i in range(n))
    slots = {}
    for i, (_, kind, n) in enumerate(items):
        slots.setdefault((i * (2 * nt - 1)) // len(items), []).append((kind, n))

    cp_x = pltpu.make_async_copy(x_hbm, x_v, wsem.at[S_X])
    cp_c = pltpu.make_async_copy(c_hbm, c_v, wsem.at[S_C])
    cp_b1 = pltpu.make_async_copy(b1_hbm, b1_v, wsem.at[S_B1])

    def wma_copy(i):
        rb, cb = divmod(i, 2 * D // PW)
        rows, cols = pl.ds(rb * RG, RG), pl.ds(cb * PW, PW)
        return pltpu.make_async_copy(
            wm_hbm.at[:, rows, cols], wm_v.at[:, rows, cols], psem.at[i])

    lows = [wma_copy(i) for i in range(NA)] + [k_copy(0, j) for j in range(nt)]
    for i in range(NL0):
        lows[i].start(priority=LO)
        if i % 8 == 7:
            (cp_c, cp_x, cp_b1)[i // 8].start(priority=HI)
    n_lo, n_hi, tot_hi = NL0, 0, 2 * (NG + WQ_AHEAD)
    for i in range(NA):
        lows[i].wait()
        ahead = NL0 + max(0, (i + 1 - (NA - NL0)) * (nt - NL0) // NL0)
        while n_lo < i + 1 + ahead:
            lows[n_lo].start(priority=LO)
            n_lo += 1
        while n_hi < min(tot_hi, ((i + 1) * tot_hi) // (NA - 2)):
            grp, rb = divmod(n_hi // 2, NG)
            wq_copy(grp, pl.ds(rb * RG, RG), (n_hi % 2) * (GC // 2), GC // 2).start(priority=HI)
            n_hi += 1
        if i == 8:
            acc_s[...] = jnp.zeros_like(acc_s)
            cp_c.wait()
            cp_x.wait()
            c = c_v[...].astype(F32)
            sc = c * (1.0 / (1.0 + jnp.exp(-c)))
            sc_s[...] = jnp.broadcast_to(sc, sc_s.shape).astype(BF16)
            xn = _layernorm(x_v[0].astype(F32))
    assert n_lo == len(lows) and n_hi == tot_hi

    mod_a = jnp.dot(sc_s[...], wm_v[:, :, 0:2 * D].reshape(D, 2 * D),
                    preferred_element_type=F32)
    h_s[...] = (xn * (1.0 + mod_a[:, D:2 * D]) + mod_a[:, 0:D]).astype(BF16)

    def q_dot(slot):
        wait_all(wq_v.at[slot], wsem.at[S_WQ + slot])
        q = jnp.dot(h_s[...], wq_v[slot].reshape(D, GC), preferred_element_type=F32)
        q_s[...] = q * (DH ** -0.5)

    def q_bcast(b):
        qb_s[b * 128:(b + 1) * 128, :] = _lane_bcast(q_s[0:1, b * 128:(b + 1) * 128])

    q_dot(0)
    for b in range(GC // 128):
        q_bcast(b)

    def wo_apply(slot, g0, g1):
        if g0 == 0:
            wait_all(wo_v.at[slot], wsem.at[S_WO + slot])
        inv_l = 1.0 / jnp.sum(av_s[DH:DH + 8, :], axis=1, keepdims=True)
        wo = wo_v[slot, g0 * 8:g1 * 8, :].astype(F32)
        a = _tree_sum(
            wo[(g - g0) * 8:(g - g0 + 1) * 8]
            * jnp.sum(av_s[g * 8:(g + 1) * 8, :], axis=1, keepdims=True)
            for g in range(g0, g1))
        acc_s[...] += a * inv_l

    def head(h, carry):
        par = lax.rem(h, 2)

        def inject(t):
            for kind, n in slots.get(t, []):
                if kind == "wq":
                    g = h * NWQ + (n + WQ_AHEAD)
                    prev = lax.div(g, NG)
                    rows = pl.ds(pl.multiple_of((g - prev * NG) * RG, RG), RG)

                    @pl.when(prev < H // GH - 1)
                    def _():
                        wq_copy(prev + 1, rows).start(priority=HI)

                    @pl.when(prev == H // GH - 1)
                    def _():
                        pltpu.make_async_copy(
                            w1_hbm.at[:, rows, :], w1_v.at[:, rows, :],
                            wsem.at[S_W1]).start(priority=HI)
                elif kind == "wo":
                    rg, ci = divmod(n, len(WO_COLS))
                    cols = pl.ds(*WO_COLS[ci])
                    pltpu.make_async_copy(
                        wo_hbm.at[pl.ds(pl.multiple_of(h * DH + rg * RG, RG), RG), cols],
                        wo_v.at[par, pl.ds(rg * RG, RG), cols],
                        wsem.at[S_WO + par]).start(priority=HI)
                else:
                    m = h * NWM + n

                    @pl.when(m < WM_TOT)
                    def _():
                        rb = lax.div(m, 4)
                        k = lax.div(rb, MR // RG)
                        rows = pl.ds(pl.multiple_of((rb - k * (MR // RG)) * RG, RG), RG)
                        cols = pl.ds(pl.multiple_of((2 + lax.rem(m, 4)) * D, 128), D)
                        pltpu.make_async_copy(
                            wm_hbm.at[k, rows, cols], wm_v.at[k, rows, cols],
                            wsem.at[S_WM]).start(priority=HI)

        qb = qb_s[pl.ds(pl.multiple_of(lax.rem(h, GH) * DH, 8), DH), :]
        mx = None
        for j in range(nt):
            k_copy(h, j).wait()
            v_copy(h, j).start(priority=LO)
            inject(j)
            pr = kbuf[j].astype(F32) * qb
            s8 = _tree_sum(pr[i * 8:(i + 1) * 8] for i in range(DH // 8))
            s = jnp.broadcast_to(jnp.sum(s8, axis=0, keepdims=True), (8, TN))
            s_s[j] = s
            mx = s if mx is None else jnp.maximum(mx, s)
            if j in WO_TICKS:
                ng = DH // 8 // len(WO_TICKS)
                g0 = WO_TICKS.index(j) * ng

                @pl.when(h > 0)
                def _():
                    wo_apply(1 - par, g0, g0 + ng)
            if j in MOD_TICKS:
                g = MOD_TICKS.index(j)

                @pl.when(h == WM_HEADS)
                def _():
                    if g == 0:
                        wait_all(wm_v.at[:, :, pl.ds(2 * D, 4 * D)], wsem.at[S_WM])
                    mod_s[:, g * D:(g + 1) * D] = jnp.dot(
                        sc_s[...], wm_v[:, :, (2 + g) * D:(3 + g) * D].reshape(D, D),
                        preferred_element_type=F32)
        row_max = jnp.max(mx, axis=1, keepdims=True)

        acc = None
        for j in range(nt):
            v_copy(h, j).wait()

            @pl.when(h < H - 1)
            def _():
                k_copy(h + 1, j).start(priority=LO)

            @pl.when(h == H - 1)
            def _():
                w2_copy(j).start(priority=LO)

            inject(nt + j)
            p = jnp.exp(s_s[j] - row_max)
            vt = vbuf[j].astype(F32)
            upd = [vt[i * 8:(i + 1) * 8] * p for i in range(DH // 8)] + [p]
            acc = upd if acc is None else [a + u for a, u in zip(acc, upd)]
            if j in Q_TICKS:
                g = Q_TICKS.index(j)

                @pl.when(jnp.logical_and(lax.rem(h, GH) == GH - 1, h < H - 1))
                def _():
                    if g == 0:
                        q_dot(lax.rem(lax.div(h, GH) + 1, 2))
                    else:
                        q_bcast(g - 1)
        for i in range(DH // 8 + 1):
            av_s[i * 8:(i + 1) * 8, :] = acc[i]
        return carry

    lax.fori_loop(0, H, head, 0)

    cp_b1.wait()
    wait_all(w1_v, wsem.at[S_W1])
    wo_apply((H - 1) % 2, 0, DH // 8)
    attn = jnp.sum(acc_s[...], axis=0, keepdims=True)
    x1 = x_v[0].astype(F32) + mod_s[0:1, 0:D] * attn
    h2 = _layernorm(x1) * (1.0 + mod_s[0:1, 2 * D:3 * D]) + mod_s[0:1, D:2 * D]
    h2 = jnp.broadcast_to(h2, (8, D)).astype(BF16)
    u = jnp.dot(h2, w1_v[...].reshape(D, FF), preferred_element_type=F32)
    u = u + b1_v[...].astype(F32).reshape(1, FF)
    sp = jnp.log1p(jnp.exp(-jnp.abs(u))) + jnp.where(u > 0, u, 0.0)
    act32 = u * jnp.tanh(sp)
    act = act32.astype(BF16)
    r_vpu = FF - W2_VPU * 128
    for b in range(W2_VPU):
        ab_s[b * 128:(b + 1) * 128, :] = _lane_bcast(
            act32[0:1, r_vpu + b * 128:r_vpu + (b + 1) * 128])

    y = jnp.zeros((8, D), F32)
    r0 = waited = 0
    for g in W2_MXU:
        r1 = r0 + g * 128
        while W2_OFF[waited] < r1:
            w2_copy(waited).wait()
            waited += 1
        y = y + jnp.dot(act[:, r0:r1], w2_v[r0:r1, :], preferred_element_type=F32)
        r0 = r1
    gb = mod_s[:, 3 * D:4 * D]
    out = jnp.broadcast_to(x1, (8, D)) + gb * y
    yv = jnp.zeros((8, D), F32)
    while r0 < FF:
        if W2_OFF[waited] <= r0:
            w2_copy(waited).wait()
            waited += 1
        for r in range(r0, W2_OFF[waited], 16):
            ab = ab_s[r - r_vpu:r - r_vpu + 16, :]
            pr = w2_v[r:r + 16, :].astype(F32) * jnp.concatenate([ab] * (D // 128), axis=1)
            yv = yv + pr[0:8] + pr[8:16]
        r0 = W2_OFF[waited]
    out = out + gb * jnp.broadcast_to(jnp.sum(yv, axis=0, keepdims=True), (8, D))
    o_ref[0] = out.astype(o_ref.dtype)[0:1]


@jax.jit
def pallas_adaLN_cond__sliding_block_cached__dense_activation_mish__decode_kernel(
    A_x: jax.Array,
    A_k_cache: jax.Array,
    A_v_cache: jax.Array,
    A_wq: jax.Array,
    A_wo: jax.Array,
    B_x: jax.Array,
    B_w1: jax.Array,
    B_b1: jax.Array,
    B_w2: jax.Array,
    c: jax.Array,
    w_mod: jax.Array,
):
    del B_x
    sk = A_k_cache.shape[2]
    win = min(4096, max(256, sk // 4))
    assert A_x.shape == (1, 1, D) and A_k_cache.shape == (1, H, sk, DH)
    assert (sk - win) % TN == 0
    nt = win // TN
    return pl.pallas_call(
        functools.partial(_kernel, win=win, start=sk - win),
        out_shape=jax.ShapeDtypeStruct((1, 1, D), A_x.dtype),
        in_specs=[pl.BlockSpec(memory_space=pl.ANY)] * 10,
        out_specs=pl.BlockSpec(memory_space=pltpu.VMEM),
        scratch_shapes=[
            pltpu.VMEM((1, 1, D), BF16),
            pltpu.VMEM((1, D), BF16),
            pltpu.VMEM((FF,), BF16),
            pltpu.VMEM((nt, DH, TN), BF16),
            pltpu.VMEM((nt, DH, TN), BF16),
            pltpu.VMEM((2, 2, HD, GC), BF16),
            pltpu.VMEM((2, DH, D), BF16),
            pltpu.VMEM((2, HD, FF), BF16),
            pltpu.VMEM((FF, D), BF16),
            pltpu.VMEM((KM, MR, 6 * D), BF16),
            pltpu.VMEM((8, D), BF16),
            pltpu.VMEM((8, D), BF16),
            pltpu.VMEM((8, GC), F32),
            pltpu.VMEM((GC, 128), F32),
            pltpu.VMEM((nt, 8, TN), F32),
            pltpu.VMEM((DH + 8, 128), F32),
            pltpu.VMEM((8, D), F32),
            pltpu.VMEM((8, 4 * D), F32),
            pltpu.VMEM((W2_VPU * 128, 128), F32),
            pltpu.SemaphoreType.DMA((nt,)),
            pltpu.SemaphoreType.DMA((nt,)),
            pltpu.SemaphoreType.DMA((NA,)),
            pltpu.SemaphoreType.DMA((9,)),
        ],
        compiler_params=pltpu.CompilerParams(
            vmem_limit_bytes=64 * 1024 * 1024,
            disable_bounds_checks=True,
            disable_semaphore_checks=True),
        name="adaln_decode",
    )(A_x, c, B_b1,
      jnp.swapaxes(A_k_cache, 2, 3), jnp.swapaxes(A_v_cache, 2, 3),
      A_wq.reshape(2, HD, H * DH), A_wo, B_w1.reshape(2, HD, FF), B_w2,
      w_mod.reshape(KM, MR, 6 * D))
```
